```python
import os as _os
_os.environ.setdefault("JAX_PLATFORMS", "cpu")
import jax
import jax.numpy as jnp

def _softmax(x, axis=-1):
    return jax.nn.softmax(x, axis=axis)
def _gelu(x):
    return jax.nn.gelu(x, approximate=True)
def _silu(x):
    return jax.nn.silu(x)
def _sigmoid(x):
    return jax.nn.sigmoid(x)
def _layernorm(x, axis=-1, eps=1e-5):
    m = jnp.mean(x, axis=axis, keepdims=True)
    v = jnp.var(x, axis=axis, keepdims=True)
    return (x - m) / jnp.sqrt(v + eps)
def _scatter_add(tgt, idx, src, axis=0):
    return tgt.at[idx].add(src)
def _segment_sum(src, seg, n):
    return jax.ops.segment_sum(src, seg, n)
class _Rng:
    def __init__(self, key):
        self._k = key
    def _next(self):
        self._k, sub = jax.random.split(self._k)
        return sub
    def normal(self, shape):
        return jax.random.normal(self._next(), shape, dtype=jnp.bfloat16)
    def randint(self, lo, hi, shape):
        return jax.random.randint(self._next(), shape, lo, hi, dtype=jnp.int32)
    def uniform(self, shape, lo=0.0, hi=1.0):
        return jax.random.uniform(self._next(), shape, jnp.bfloat16, lo, hi)
    def permutation(self, n):
        return jax.random.permutation(self._next(), n)


kernel_name = 'concat_heads__linear_kernel_hedgehog__ssm_conv_s5__prompt'

def setup_inputs():
    _rng = _Rng(jax.random.key(int.from_bytes(__import__("os").urandom(4), "little")))
    _w = (lambda a: (lambda t: t.astype(jnp.bfloat16) if jnp.issubdtype(t.dtype, jnp.floating) else t)(jnp.asarray(a)))
    def _A_setup():
        B, S, D, H = 1, 2048, 640, 32
        Dh = D // H
        return {
            "x": _w((lambda *s: _rng.normal(s) * 0.4)(B, S, D)),
            "wqkv": _w((lambda *s: _rng.normal(s) * 0.4)(D, 3 * D)),
            "w_phi": _w((lambda *s: _rng.normal(s) * 0.4)(H, Dh, Dh) * (Dh ** -0.5)),
            "wo": _w((lambda *s: _rng.normal(s) * 0.05)(D, D)),
        }
    _A_in = _A_setup()

    def _B_setup():
        B, S, D = 1, 2048, 640
        P = D
        Lambda_re = -0.5 * jnp.exp((lambda *s: _rng.normal(s) * 0.8)(P))
        Lambda_im = (lambda *s: _rng.normal(s) * 0.8)(P) * 1.0
        B_re = (lambda *s: _rng.normal(s) * 0.8)(P, D) * (D ** -0.5)
        B_im = (lambda *s: _rng.normal(s) * 0.8)(P, D) * (D ** -0.5)
        C_re = (lambda *s: _rng.normal(s) * 0.8)(D, P) * (P ** -0.5)
        C_im = (lambda *s: _rng.normal(s) * 0.8)(D, P) * (P ** -0.5)
        log_dt = (lambda *s: _rng.normal(s) * 0.8)(P) * 0.3 - 2.0
        Dskip = (lambda *s: _rng.normal(s) * 0.8)(D)
        return {
            "x": _w((lambda *s: _rng.normal(s) * 0.05)(B, S, D)),
            "Lambda_re": _w(Lambda_re),
            "Lambda_im": _w(Lambda_im),
            "B_re": _w(B_re),
            "B_im": _w(B_im),
            "C_re": _w(C_re),
            "C_im": _w(C_im),
            "log_dt": _w(log_dt),
            "Dskip": _w(Dskip),
        }
    _B_in = _B_setup()

    return {
        "A_x": _A_in["x"],
        "A_wqkv": _A_in["wqkv"],
        "A_w_phi": _A_in["w_phi"],
        "A_wo": _A_in["wo"],
        "B_x": _B_in["x"],
        "B_Lambda_re": _B_in["Lambda_re"],
        "B_Lambda_im": _B_in["Lambda_im"],
        "B_B_re": _B_in["B_re"],
        "B_B_im": _B_in["B_im"],
        "B_C_re": _B_in["C_re"],
        "B_C_im": _B_in["C_im"],
        "B_log_dt": _B_in["log_dt"],
        "B_Dskip": _B_in["Dskip"],
    }

def reference(A_x, A_wqkv, A_w_phi, A_wo, B_x, B_Lambda_re, B_Lambda_im, B_B_re, B_B_im, B_C_re, B_C_im, B_log_dt, B_Dskip):
    def _A_ref(x, wqkv, w_phi, wo):
        B, S, D = x.shape
        H = 32; Dh = D // H
        qkv = (lambda x, *d: x.transpose(*d))((x @ wqkv).reshape(B, S, 3, H, Dh), 2, 0, 3, 1, 4)
        q, k, v = qkv[0], qkv[1], qkv[2]
        pq = jnp.einsum("bhsd,hdf->bhsf", q, w_phi)
        pk = jnp.einsum("bhsd,hdf->bhsf", k, w_phi)
        phi_q = jnp.concatenate([_softmax(pq, axis=-1), _softmax(-pq, axis=-1)], axis=-1)
        phi_k = jnp.concatenate([_softmax(pk, axis=-1), _softmax(-pk, axis=-1)], axis=-1)
        kv = jnp.einsum("bhsf,bhsd->bhfd", phi_k, v)
        z  = jnp.einsum("bhsf->bhf", phi_k)
        num = jnp.einsum("bhqf,bhfd->bhqd", phi_q, kv)
        den = jnp.einsum("bhqf,bhf->bhq", phi_q, z)[..., None] + 1e-6
        o = num / den
        return (lambda x, *d: x.transpose(*d))(o, 0, 2, 1, 3).reshape(B, S, D) @ wo

    def _B_ref(x, Lambda_re, Lambda_im, B_re, B_im, C_re, C_im, log_dt, Dskip):
        Bsz, L, H = x.shape
        Lam = Lambda_re + 1j * Lambda_im
        Bmat = B_re + 1j * B_im
        Cmat = C_re + 1j * C_im
        dt = jnp.exp(log_dt)
        Lam_bar = jnp.exp(dt * Lam)
        B_bar = ((Lam_bar - 1.0) / Lam)[:, None] * Bmat
        Bu = jnp.einsum("bld,pd->blp", x + 0j, B_bar)
        h = jnp.zeros_like(Bu[:, 0, :])
        hs = []
        for t in range(L):
            h = Lam_bar[None, :] * h + Bu[:, t, :]
            hs.append(h)
        hseq = jnp.stack(hs, 1)
        y = 2.0 * jnp.einsum("blp,dp->bld", hseq, Cmat).real + x * Dskip[None, None, :]
        return y

    a = _A_ref(A_x, A_wqkv, A_w_phi, A_wo)
    b = _B_ref(B_x, B_Lambda_re, B_Lambda_im, B_B_re, B_B_im, B_C_re, B_C_im, B_log_dt, B_Dskip)
    return jnp.concatenate([a, b], axis=-1)
```

```python
import functools

import jax
import jax.numpy as jnp
from jax import lax
import jax.experimental.pallas as pl
import jax.experimental.pallas.tpu as pltpu

S = 2048
D = 640
H = 32
DH = 20
NG = 8
GR = 80

F32 = jnp.float32
BF16 = jnp.bfloat16
NT = (((1,), (1,)), ((), ()))
NN = (((1,), (0,)), ((), ()))
TN = (((0,), (0,)), ((), ()))


def _dot(a, b, dims=NN):
    return lax.dot_general(a, b, dims, preferred_element_type=F32)


def _fdiv(x, d):
    return jnp.floor((x.astype(F32) + 0.5) * (1.0 / d)).astype(jnp.int32)


def _tile_rows(i):
    half, j = divmod(i, 5)
    g_lo = (128 * j) // 160
    g_hi = (128 * j + 127) // 160
    return half * 320 + g_lo * GR, (g_hi - g_lo + 1) * GR


def _tile_offsets():
    offs, o = [], 0
    for i in range(10):
        offs.append(o)
        o += _tile_rows(i)[1]
    return offs


TILE_OFF = _tile_offsets()


def _cmul(ar, ai, br, bi):
    return ar * br - ai * bi, ar * bi + ai * br


def _kernel(xa_ref, wqkv_ref, wphi_ref, wo_ref, xb_ref, lre_ref, lim_ref,
            bre_ref, bim_ref, cre_ref, cim_ref, ldt_ref, dsk_ref,
            out_ref,
            wk_s, wq_s, c_s, lam_s, kv_s, kvb_s, z_s, w2_s, *, SB, TB):
    lre = lre_ref[...].astype(F32).reshape(1, D)
    lim = lim_ref[...].astype(F32).reshape(1, D)
    dt = jnp.exp(ldt_ref[...].astype(F32).reshape(1, D)).astype(BF16).astype(F32)
    ar = dt * lre
    ai = dt * lim
    kk = (lax.broadcasted_iota(jnp.int32, (8, D), 0) + 1).astype(F32)
    mag = jnp.exp(kk * ar)
    t_re = mag * jnp.cos(kk * ai)
    t_im = mag * jnp.sin(kk * ai)
    row = lax.broadcasted_iota(jnp.int32, (8, D), 0)
    for n, sh in enumerate((1, 2, 4)):
        keep = row >= sh
        lam_s[2 * n] = jnp.where(keep, jnp.broadcast_to(t_re[sh - 1:sh], (8, D)), 0.0)
        lam_s[2 * n + 1] = jnp.where(keep, jnp.broadcast_to(t_im[sh - 1:sh], (8, D)), 0.0)
    lam_s[6] = t_re
    lam_s[7] = t_im
    l_re = t_re[0:1]
    l_im = t_im[0:1]
    inv = 1.0 / (lre * lre + lim * lim)
    nr = l_re - 1.0
    co_re = (nr * lre + l_im * lim) * inv
    co_im = (l_im * lre - nr * lim) * inv
    for r in range(5):
        sl = pl.ds(128 * r, 128)
        cr = cre_ref[sl, :].astype(F32)
        ci = cim_ref[sl, :].astype(F32)
        c_s[sl, 0:D] = (2.0 * (co_re * cr - co_im * ci)).astype(BF16)
        c_s[sl, D:2 * D] = (-2.0 * (co_re * ci + co_im * cr)).astype(BF16)
    dsk = dsk_ref[...].astype(F32).reshape(1, D)

    w2_s[...] = jnp.zeros(w2_s.shape, F32)
    for h in range(H):
        w2_s[pl.ds(DH * h, DH), 0:DH] = wphi_ref[h].astype(F32)
    w2 = w2_s[...].astype(BF16)
    r_i = lax.broadcasted_iota(jnp.int32, (D, 128), 0)
    c_i = lax.broadcasted_iota(jnp.int32, (D, 128), 1)
    g_r = _fdiv(r_i, GR)
    f_r = _fdiv(r_i - g_r * GR, 4)
    h_r = 4 * g_r + (r_i & 3)
    e_t = jnp.where(f_r == c_i, 1.0, 0.0).astype(BF16)
    phit = []
    for kt in range(5):
        rep = _dot(e_t, w2[128 * kt:128 * (kt + 1)], NT)
        h_c = _fdiv(c_i + 128 * kt, DH)
        phit.append(jnp.where(h_r == h_c, rep, 0.0).astype(BF16))

    def fold(col0):
        acc = [None] * NG
        for kt in range(5):
            g_lo = (128 * kt) // GR
            g_hi = (128 * kt + 127) // GR
            part = _dot(phit[kt][g_lo * GR:(g_hi + 1) * GR],
                        wqkv_ref[:, col0 + 128 * kt:col0 + 128 * (kt + 1)], NT)
            for g in range(g_lo, g_hi + 1):
                p = part[(g - g_lo) * GR:(g - g_lo + 1) * GR]
                acc[g] = p if acc[g] is None else acc[g] + p
        return acc

    for g, a in enumerate(fold(0)):
        wq_s[g * GR:(g + 1) * GR, :] = a.astype(BF16)
    for g, a in enumerate(fold(D)):
        wk_s[g * GR:(g + 1) * GR, :] = a.astype(BF16)
    wk_s[D:2 * D, :] = wqkv_ref[:, 2 * D:3 * D].astype(F32).T.astype(BF16)
    kv_s[...] = jnp.zeros(kv_s.shape, F32)
    z_s[...] = jnp.zeros(z_s.shape, F32)

    def features(p):
        ps = [p[8 * k:8 * k + 8] for k in range(10)]
        mx = functools.reduce(jnp.maximum, ps)
        mn = functools.reduce(jnp.minimum, ps)
        mx = jnp.maximum(mx, pltpu.roll(mx, 4, 0))
        mn = jnp.minimum(mn, pltpu.roll(mn, 4, 0))
        ep = [jnp.exp(q - mx) for q in ps]
        en = [jnp.exp(mn - q) for q in ps]
        sp = functools.reduce(jnp.add, ep)
        sn = functools.reduce(jnp.add, en)
        sp = sp + pltpu.roll(sp, 4, 0)
        sn = sn + pltpu.roll(sn, 4, 0)
        return ep, en, sp, sn

    def k_side(i):
        x = xa_ref[pl.ds(pl.multiple_of(i * SB, SB), SB), :]
        pkv = _dot(wk_s[...], x, NT)
        vt = pkv[D:].astype(BF16)
        rows = []
        for g in range(NG):
            ep, en, sp, sn = features(pkv[g * GR:(g + 1) * GR])
            rp = 1.0 / sp
            rn = 1.0 / sn
            rows += [e * rp for e in ep] + [e * rn for e in en]
        phi = jnp.concatenate(rows, axis=0)
        zs = phi[:, 0:128]
        for c in range(1, SB // 128):
            zs = zs + phi[:, 128 * c:128 * (c + 1)]
        z_s[...] += zs
        phib = phi.astype(BF16)
        for t in range(10):
            r0, nr_ = _tile_rows(t)
            kv_s[TILE_OFF[t]:TILE_OFF[t] + nr_, :] += _dot(
                vt[r0:r0 + nr_], phib[128 * t:128 * (t + 1)], NT)

    def finalize_kv():
        z = jnp.sum(z_s[...], axis=1, keepdims=True)
        z_s[...] = jnp.broadcast_to(z, z_s.shape)
        for t in range(10):
            r0, nr_ = _tile_rows(t)
            rr = lax.broadcasted_iota(jnp.int32, (nr_, 128), 0) + r0
            cc = lax.broadcasted_iota(jnp.int32, (nr_, 128), 1) + 128 * t
            h_row = _fdiv(rr, DH)
            h_col = 4 * _fdiv(cc, 160) + (cc & 3)
            kvb_s[TILE_OFF[t]:TILE_OFF[t] + nr_, :] = jnp.where(
                h_row == h_col, kv_s[TILE_OFF[t]:TILE_OFF[t] + nr_, :], 0.0).astype(BF16)

    def q_side(i):
        r0_ = pl.multiple_of(i * SB, SB)
        x = xa_ref[pl.ds(r0_, SB), :]
        pq = _dot(wq_s[...], x, NT)
        rows = []
        nl = SB // 128
        for g in range(NG):
            ep, en, sp, sn = features(pq[g * GR:(g + 1) * GR])
            zb = z_s[g * 160:(g + 1) * 160, :]
            zb = jnp.concatenate([zb] * nl, axis=1) if nl > 1 else zb
            dp = functools.reduce(jnp.add, [ep[k] * zb[8 * k:8 * k + 8] for k in range(10)])
            dn = functools.reduce(jnp.add, [en[k] * zb[80 + 8 * k:88 + 8 * k] for k in range(10)])
            dd = dp / sp + dn / sn
            den = dd + pltpu.roll(dd, 4, 0) + 1e-6
            rp = 1.0 / (sp * den)
            rn = 1.0 / (sn * den)
            rows += [e * rp for e in ep] + [e * rn for e in en]
        phib = jnp.concatenate(rows, axis=0).astype(BF16)
        acc = [None] * NG
        for t in range(10):
            r0, nr_ = _tile_rows(t)
            part = _dot(kvb_s[TILE_OFF[t]:TILE_OFF[t] + nr_, :], phib[128 * t:128 * (t + 1)])
            for k in range(nr_ // GR):
                g = r0 // GR + k
                p = part[k * GR:(k + 1) * GR]
                acc[g] = p if acc[g] is None else acc[g] + p
        ot = jnp.concatenate(acc, axis=0).astype(BF16)
        out_ref[pl.ds(r0_, SB), 0:D] = _dot(ot, wo_ref[...], TN)

    def ssm(j, carry):
        r0_ = pl.multiple_of(j * TB, TB)
        xb = xb_ref[pl.ds(r0_, TB), :]
        w_re = _dot(xb, bre_ref[...], NT)
        w_im = _dot(xb, bim_ref[...], NT)
        c_re, c_im = carry
        outs_re, outs_im = [], []
        for r in range(TB // 8):
            u_re = w_re[8 * r:8 * r + 8]
            u_im = w_im[8 * r:8 * r + 8]
            for n, sh in enumerate((1, 2, 4)):
                m_re = lam_s[2 * n]
                m_im = lam_s[2 * n + 1]
                s_re = pltpu.roll(u_re, sh, 0)
                s_im = pltpu.roll(u_im, sh, 0)
                d_re, d_im = _cmul(m_re, m_im, s_re, s_im)
                u_re = u_re + d_re
                u_im = u_im + d_im
            d_re, d_im = _cmul(lam_s[6], lam_s[7], c_re, c_im)
            u_re = u_re + d_re
            u_im = u_im + d_im
            c_re = jnp.broadcast_to(u_re[7:8], (8, D))
            c_im = jnp.broadcast_to(u_im[7:8], (8, D))
            outs_re.append(u_re)
            outs_im.append(u_im)
        s = jnp.concatenate([jnp.concatenate(outs_re, 0), jnp.concatenate(outs_im, 0)],
                            axis=1).astype(BF16)
        y = _dot(s, c_s[...], NT) + xb.astype(F32) * dsk
        out_ref[pl.ds(r0_, TB), D:2 * D] = y
        return c_re, c_im

    n1 = S // SB
    assert 2 * n1 * TB == S
    zero = jnp.zeros((8, D), F32)

    def body1(i, carry):
        k_side(i)
        return ssm(i, carry)

    carry = lax.fori_loop(0, n1, body1, (zero, zero))
    finalize_kv()

    def body2(i, carry):
        q_side(i)
        return ssm(i + n1, carry)

    lax.fori_loop(0, n1, body2, carry)


SB_ = 256


@jax.jit
def pallas_concat_heads__linear_kernel_hedgehog__ssm_conv_s5__prompt_kernel(
    A_x, A_wqkv, A_w_phi, A_wo, B_x, B_Lambda_re, B_Lambda_im, B_B_re, B_B_im,
    B_C_re, B_C_im, B_log_dt, B_Dskip,
):
    out = pl.pallas_call(
        functools.partial(_kernel, SB=SB_, TB=SB_ // 2),
        out_shape=jax.ShapeDtypeStruct((S, 2 * D), F32),
        scratch_shapes=[
            pltpu.VMEM((2 * D, D), BF16),
            pltpu.VMEM((D, D), BF16),
            pltpu.VMEM((D, 2 * D), BF16),
            pltpu.VMEM((8, 8, D), F32),
            pltpu.VMEM((2 * D, 128), F32),
            pltpu.VMEM((2 * D, 128), BF16),
            pltpu.VMEM((2 * D, 128), F32),
            pltpu.VMEM((D, 128), F32),
        ],
        compiler_params=pltpu.CompilerParams(vmem_limit_bytes=100 * 1024 * 1024),
        name="hedgehog_s5",
    )(A_x.reshape(S, D), A_wqkv, A_w_phi, A_wo, B_x.reshape(S, D), B_Lambda_re,
      B_Lambda_im, B_B_re, B_B_im, B_C_re, B_C_im, B_log_dt, B_Dskip)
    return out.reshape(1, S, 2 * D)
```

```python
import functools

import jax
import jax.numpy as jnp
from jax import lax
import jax.experimental.pallas as pl
import jax.experimental.pallas.tpu as pltpu

S = 2048
D = 640
H = 32
DH = 20
NG = 8
GR = 80

F32 = jnp.float32
BF16 = jnp.bfloat16
NT = (((1,), (1,)), ((), ()))
NN = (((1,), (0,)), ((), ()))
TN = (((0,), (0,)), ((), ()))


def _dot(a, b, dims=NN):
    return lax.dot_general(a, b, dims, preferred_element_type=F32)


def _ld(ref, r0, r1, cols=slice(None)):
    return pltpu.bitcast(ref[r0 // 2:r1 // 2, cols], BF16)


def _st(ref, r0, val, cols=slice(None)):
    ref[r0 // 2:(r0 + val.shape[0]) // 2, cols] = pltpu.bitcast(val.astype(BF16), jnp.int32)


def _fdiv(x, d):
    return jnp.floor((x.astype(F32) + 0.5) * (1.0 / d)).astype(jnp.int32)


def _tile_rows(i):
    half, j = divmod(i, 5)
    g_lo = (128 * j) // 160
    g_hi = (128 * j + 127) // 160
    return half * 320 + g_lo * GR, (g_hi - g_lo + 1) * GR


def _tile_offsets():
    offs, o = [], 0
    for i in range(10):
        offs.append(o)
        o += _tile_rows(i)[1]
    return offs


TILE_OFF = _tile_offsets()


def _loop(n, wait, body, state, unroll):
    def step(k, st):
        for u in range(unroll):
            wait(k * unroll + u)
        for u in range(unroll):
            st = body(k * unroll + u, st)
        return st
    if unroll == n:
        return step(0, state)
    return lax.fori_loop(0, n // unroll, step, state)


def _mult(x, m):
    return x if isinstance(x, int) else pl.multiple_of(x, m)


def _kernel(xa_hbm, wqkv_hbm, wphi_hbm, wo_hbm, xb_hbm, lre_hbm, lim_hbm,
            bre_hbm, bim_hbm, cre_hbm, cim_hbm, ldt_hbm, dsk_hbm,
            out_hbm,
            xa_s, xb_s, wqkv_s, wo_s, b_s, craw_s, wphi_s, p0_s, p1_s, p2_s, p3_s,
            wk_s, wq_s, c_s, phit_s, lam_s, dsk_s, kv_s, kvb_s, z_s,
            b2_s, zb_s, ya_s, yb_s, isem, xsem, osem, *, SB, T, TA, U1, U2, JS, JB, KSPLIT):
    n1 = S // SB
    T0 = S - 2 * n1 * T

    par_in = (lre_hbm, lim_hbm, ldt_hbm, dsk_hbm)
    par_s = (p0_s, p1_s, p2_s, p3_s)
    par_cp = [pltpu.make_async_copy(r, par_s[k], isem.at[k]) for k, r in enumerate(par_in)]
    wphi_cp = pltpu.make_async_copy(wphi_hbm, wphi_s, isem.at[4])
    xa_cp0 = pltpu.make_async_copy(xb_hbm.at[0:T0], xb_s.at[0:T0], isem.at[5])
    b_cp0, b_cp1 = [], []
    for k, r in enumerate((bre_hbm, bim_hbm)):
        b_cp0.append(pltpu.make_async_copy(
            r.at[0:128 * JB], b_s.at[D * k:D * k + 128 * JB], isem.at[7 + k]))
        b_cp1.append(pltpu.make_async_copy(
            r.at[128 * JB:D], b_s.at[D * k + 128 * JB:D * (k + 1)], isem.at[9 + k]))
    c_cp = [pltpu.make_async_copy(r, craw_s.at[k], isem.at[11 + k])
            for k, r in enumerate((cre_hbm, cim_hbm))]
    wqkv_cp = pltpu.make_async_copy(wqkv_hbm, wqkv_s, isem.at[13])
    wo_cp = pltpu.make_async_copy(wo_hbm, wo_s, isem.at[14])

    def xa_cp(i):
        r = pl.ds(_mult(i * SB, SB), SB)
        return pltpu.make_async_copy(xa_hbm.at[r], xa_s.at[r], xsem.at[i])

    def ssm_rows(blk):
        return pl.ds(_mult(T0 + blk * T, 16), T)

    def xb_cp(blk):
        r = ssm_rows(blk)
        return pltpu.make_async_copy(xb_hbm.at[r], xb_s.at[r], xsem.at[n1 + blk])

    for cp in par_cp + [wphi_cp, xa_cp0] + b_cp0:
        cp.start()

    for cp in par_cp:
        cp.wait()
    for cp in b_cp1:
        cp.start()
    lre = par_s[0][...].astype(F32).reshape(1, D)
    lim = par_s[1][...].astype(F32).reshape(1, D)
    dt = jnp.exp(par_s[2][...].astype(F32).reshape(1, D)).astype(BF16).astype(F32)
    dsk_s[...] = jnp.broadcast_to(par_s[3][...].astype(F32).reshape(1, D), (8, D))
    ar = dt * lre
    ai = dt * lim
    kk = (lax.broadcasted_iota(jnp.int32, (8, D), 0) + 1).astype(F32)
    mag = jnp.exp(kk * ar)
    t_re = mag * jnp.cos(kk * ai)
    t_im = mag * jnp.sin(kk * ai)
    row = lax.broadcasted_iota(jnp.int32, (8, D), 0)
    for n, (sh, keep) in enumerate(((1, row == 0), (1, row >= 1), (2, row >= 2), (4, row >= 4))):
        lam_s[2 * n] = jnp.where(keep, jnp.broadcast_to(t_re[sh - 1:sh], (8, D)), 0.0)
        lam_s[2 * n + 1] = jnp.where(keep, jnp.broadcast_to(t_im[sh - 1:sh], (8, D)), 0.0)
    l_re = t_re[0:1]
    l_im = t_im[0:1]
    inv = 1.0 / (lre * lre + lim * lim)
    nr = l_re - 1.0
    co_re = 2.0 * (nr * lre + l_im * lim) * inv
    co_im = 2.0 * (l_im * lre - nr * lim) * inv

    wphi_cp.wait()
    for cp in c_cp:
        cp.start()

    def prep_phi():
        lcat = jnp.concatenate([wphi_s[d].astype(F32) for d in range(DH)], axis=1)
        lcat = lcat.astype(BF16)
        r_i = lax.broadcasted_iota(jnp.int32, (GR, 128), 0)
        l_i = lax.broadcasted_iota(jnp.int32, (GR, 128), 1)
        e_g = jnp.where((r_i >> 2)[:, 0:DH] == l_i[:, 0:DH], 1.0, 0.0).astype(BF16)
        hl_r = r_i & 3
        k_i = lax.broadcasted_iota(jnp.int32, (D, 128), 0)
        for ct in range(5):
            cc = lax.broadcasted_iota(jnp.int32, (8, 128), 1) + 128 * ct
            h_c = _fdiv(cc, DH)
            tgt = 32 * (cc - DH * h_c) + h_c
            pm = jnp.where(k_i == tgt[0:1], 1.0, 0.0).astype(BF16)
            x_t = _dot(lcat, pm).astype(BF16)
            rep = _dot(e_g, x_t)
            for g in range((128 * ct) // GR, (128 * ct + 127) // GR + 1):
                _st(phit_s, g * GR, jnp.where(hl_r + 4 * g == h_c[0:1], rep, 0.0),
                    slice(128 * ct, 128 * (ct + 1)))

    prep_phi()

    def fold(col0, dst):
        acc = [None] * NG
        for kt in range(5):
            g_lo = (128 * kt) // GR
            g_hi = (128 * kt + 127) // GR
            part = _dot(_ld(phit_s, g_lo * GR, (g_hi + 1) * GR, slice(128 * kt, 128 * (kt + 1))),
                        wqkv_s[:, col0 + 128 * kt:col0 + 128 * (kt + 1)], NT)
            for g in range(g_lo, g_hi + 1):
                p = part[(g - g_lo) * GR:(g - g_lo + 1) * GR]
                acc[g] = p if acc[g] is None else acc[g] + p
        for g, a in enumerate(acc):
            _st(dst, g * GR, a)

    def prep_c():
        for j in range(5):
            cs = slice(128 * j, 128 * (j + 1))
            cr_ = co_re[:, cs]
            ci_ = co_im[:, cs]
            for r in range(5):
                rs = slice(128 * r, 128 * (r + 1))
                a = craw_s[0, rs, cs].astype(F32)
                b = craw_s[1, rs, cs].astype(F32)
                _st(c_s, 128 * r, cr_ * a - ci_ * b, slice(256 * j, 256 * j + 128))
                _st(c_s, 128 * r, -(cr_ * b + ci_ * a), slice(256 * j + 128, 256 * j + 256))

    def features(p):
        ps = [p[8 * k:8 * k + 8] for k in range(10)]
        mx = functools.reduce(jnp.maximum, ps)
        mn = functools.reduce(jnp.minimum, ps)
        mx = jnp.maximum(mx, pltpu.roll(mx, 4, 0))
        mn = jnp.minimum(mn, pltpu.roll(mn, 4, 0))
        ep = [jnp.exp(q - mx) for q in ps]
        en = [jnp.exp(mn - q) for q in ps]
        sp = functools.reduce(jnp.add, ep)
        sn = functools.reduce(jnp.add, en)
        sp = sp + pltpu.roll(sp, 4, 0)
        sn = sn + pltpu.roll(sn, 4, 0)
        return ep, en, sp, sn

    def k_proj(i):
        x = xa_s[pl.ds(_mult(i * SB, SB), SB), :]
        return _dot(_ld(wk_s, 0, 2 * D), x, NT)

    def k_side(pkv, mid):
        vt = pkv[D:].astype(BF16)
        rows = []
        for g in range(NG):
            ep, en, sp, sn = features(pkv[g * GR:(g + 1) * GR])
            rp = 1.0 / sp
            rn = 1.0 / sn
            rows += [e * rp for e in ep] + [e * rn for e in en]
        phi = jnp.concatenate(rows, axis=0)
        zs = phi[:, 0:128]
        for c in range(1, SB // 128):
            zs = zs + phi[:, 128 * c:128 * (c + 1)]
        z_s[...] += zs
        phib = phi.astype(BF16)
        mid()
        for t in range(10):
            r0, nr_ = _tile_rows(t)
            kv_s[TILE_OFF[t]:TILE_OFF[t] + nr_, :] += _dot(
                vt[r0:r0 + nr_], phib[128 * t:128 * (t + 1)], NT)

    def finalize_kv():
        z = jnp.sum(z_s[...], axis=1, keepdims=True)
        zb_s[...] = jnp.broadcast_to(z, z_s.shape)
        for t in range(10):
            r0, nr_ = _tile_rows(t)
            rr = lax.broadcasted_iota(jnp.int32, (nr_, 128), 0) + r0
            cc = lax.broadcasted_iota(jnp.int32, (nr_, 128), 1) + 128 * t
            h_row = _fdiv(rr, DH)
            h_col = 4 * _fdiv(cc, 160) + (cc & 3)
            _st(kvb_s, TILE_OFF[t], jnp.where(
                h_row == h_col, kv_s[TILE_OFF[t]:TILE_OFF[t] + nr_, :], 0.0))

    def q_proj(i):
        x = xa_s[pl.ds(_mult(i * SB, SB), SB), :]
        return _dot(_ld(wq_s, 0, D), x, NT)

    def q_side(i, pq):
        r0_ = _mult(i * SB, SB)
        rows = []
        nl = SB // 128
        for g in range(NG):
            ep, en, sp, sn = features(pq[g * GR:(g + 1) * GR])
            zb = zb_s[g * 160:(g + 1) * 160, :]
            zb = jnp.concatenate([zb] * nl, axis=1) if nl > 1 else zb
            dp = functools.reduce(jnp.add, [ep[k] * zb[8 * k:8 * k + 8] for k in range(10)])
            dn = functools.reduce(jnp.add, [en[k] * zb[80 + 8 * k:88 + 8 * k] for k in range(10)])
            dd = dp / sp + dn / sn
            den = dd + pltpu.roll(dd, 4, 0) + 1e-6
            rp = 1.0 / (sp * den)
            rn = 1.0 / (sn * den)
            rows += [e * rp for e in ep] + [e * rn for e in en]
        phib = jnp.concatenate(rows, axis=0).astype(BF16)
        acc = [None] * NG
        for t in range(10):
            r0, nr_ = _tile_rows(t)
            part = _dot(_ld(kvb_s, TILE_OFF[t], TILE_OFF[t] + nr_), phib[128 * t:128 * (t + 1)])
            for k in range(nr_ // GR):
                g = r0 // GR + k
                p = part[k * GR:(k + 1) * GR]
                acc[g] = p if acc[g] is None else acc[g] + p
        ot = jnp.concatenate(acc, axis=0).astype(BF16)
        for c in range(nl):
            rc = pl.ds(_mult(r0_ + 128 * c, 128), 128)
            ya_s[rc, :] = _dot(ot[:, 128 * c:128 * (c + 1)], wo_s[...], TN)
            pltpu.make_async_copy(ya_s.at[rc], out_hbm.at[rc, pl.ds(0, D)], osem).start()

    def ssm_w(xb, j):
        return _dot(xb, _ld(b2_s, 256 * j, 256 * (j + 1)), NT)

    def pack_b(j):
        _st(b2_s, 256 * j, b_s[128 * j:128 * (j + 1), :])
        _st(b2_s, 256 * j + 128, b_s[D + 128 * j:D + 128 * (j + 1), :])

    def ssm_scan(w, j, carry):
        tb = w.shape[0]
        cs = slice(128 * j, 128 * (j + 1))
        tab = [lam_s[n, :, cs] for n in range(8)]
        c_re, c_im = carry[2 * j], carry[2 * j + 1]
        o_re, o_im = [], []
        for r in range(tb // 8):
            u_re = w[8 * r:8 * r + 8, 0:128]
            u_im = w[8 * r:8 * r + 8, 128:256]
            for n, sh in enumerate((1, 1, 2, 4)):
                m_re, m_im = tab[2 * n], tab[2 * n + 1]
                s_re = pltpu.roll(c_re if n == 0 else u_re, sh, 0)
                s_im = pltpu.roll(c_im if n == 0 else u_im, sh, 0)
                u_re = u_re + (m_re * s_re - m_im * s_im)
                u_im = u_im + (m_re * s_im + m_im * s_re)
            c_re, c_im = u_re, u_im
            o_re.append(u_re)
            o_im.append(u_im)
        carry = carry[:2 * j] + (c_re, c_im) + carry[2 * j + 2:]
        return [jnp.concatenate(o_re, 0).astype(BF16),
                jnp.concatenate(o_im, 0).astype(BF16)], carry

    def ssm_scan_all(ws, carry):
        s_tiles = []
        for j in range(5):
            st, carry = ssm_scan(ws[j], j, carry)
            s_tiles += st
        return jnp.concatenate(s_tiles, axis=1), carry

    def ssm_back(s, rows):
        y = xb_s[rows, :].astype(F32) * dsk_s[0:1, :]
        if KSPLIT and isinstance(rows.start, int):
            for j in range(5):
                y = y + _dot(s[:, 256 * j:256 * (j + 1)], _ld(c_s, 0, D, slice(256 * j, 256 * (j + 1))), NT)
        else:
            y = y + _dot(s, _ld(c_s, 0, D), NT)
        yb_s[rows, :] = y

    def ssm_out(rows):
        pltpu.make_async_copy(yb_s.at[rows], out_hbm.at[rows, pl.ds(D, D)], osem).start()

    zero = jnp.zeros((8, 128), F32)
    carry = (zero,) * 10
    rows0 = pl.ds(0, T0)
    xa_cp0.wait()
    for cp in b_cp0:
        cp.wait()
    wqkv_cp.start()
    xb0 = xb_s[rows0, :]
    for j in range(JB):
        pack_b(j)
    w0 = [ssm_w(xb0, j) for j in range(JB)]
    for cp in b_cp1:
        cp.wait()
    xa_cp(0).start()
    xb_cp(0).start()
    for j in range(JB, 5):
        pack_b(j)
    w0 += [ssm_w(xb0, j) for j in range(JB, 5)]
    parts = [(0, TA), (TA, T0)]
    st = {}

    def scan_part(j, p, carry):
        lo, hi = parts[p]
        st[j, p], carry = ssm_scan(w0[j][lo:hi], j, carry)
        return carry

    early = [(j, p) for j in range(5) for p in range(2) if j < JS[p]]
    for j, p in early:
        carry = scan_part(j, p, carry)
    for cp in c_cp:
        cp.wait()
    prep_c()
    for j in range(5):
        for p in range(2):
            if (j, p) not in early:
                carry = scan_part(j, p, carry)
    for p, (lo, hi) in enumerate(parts):
        ssm_back(jnp.concatenate([t for j in range(5) for t in st[j, p]], axis=1),
                 pl.ds(lo, hi - lo))
    kv_s[...] = jnp.zeros(kv_s.shape, F32)
    z_s[...] = jnp.zeros(z_s.shape, F32)
    ssm_out(pl.ds(0, T0))
    wqkv_cp.wait()
    wo_cp.start()
    for i in range(1, n1):
        xa_cp(i).start()
        xb_cp(i).start()
    fold(0, wq_s)
    fold(D, wk_s)
    _st(wk_s, D, wqkv_s[:, 2 * D:3 * D].T)
    for i in range(n1):
        xb_cp(n1 + i).start()

    def wait1(i):
        xa_cp(i).wait()
        xb_cp(i).wait()

    def body1(i, carry):
        rows = ssm_rows(i)
        ws = [ssm_w(xb_s[rows, :], j) for j in range(5)]
        pkv = k_proj(i)
        s, carry = ssm_scan_all(ws, carry)
        ssm_back(s, rows)
        k_side(pkv, lambda: None)
        ssm_out(rows)
        return carry

    carry = _loop(n1, wait1, body1, carry, U1)
    wo_cp.wait()

    def wait2(i):
        xb_cp(i + n1).wait()

    def body2(i, carry):
        rows = ssm_rows(i + n1)
        ws = [ssm_w(xb_s[rows, :], j) for j in range(5)]
        pq = q_proj(i)
        finalize_kv()
        s, carry = ssm_scan_all(ws, carry)
        ssm_back(s, rows)
        ssm_out(rows)
        q_side(i, pq)
        return carry

    _loop(n1, wait2, body2, carry, U2)
    pltpu.make_async_copy(out_hbm, out_hbm, osem).wait()


SB = 512
T = 208
TA = 192
U1 = 1
U2 = 1
JS = (3, 2)
JB = 2
KSPLIT = 1


@jax.jit
def pallas_concat_heads__linear_kernel_hedgehog__ssm_conv_s5__prompt_kernel(
    A_x, A_wqkv, A_w_phi, A_wo, B_x, B_Lambda_re, B_Lambda_im, B_B_re, B_B_im,
      B_C_re, B_C_im, B_log_dt, B_Dskip):
    n1 = S // SB
    out = pl.pallas_call(
        functools.partial(_kernel, SB=SB, T=T, TA=TA, U1=U1, U2=U2, JS=JS, JB=JB, KSPLIT=KSPLIT),
        out_shape=jax.ShapeDtypeStruct((S, 2 * D), F32),
        in_specs=[pl.BlockSpec(memory_space=pl.ANY)] * 13,
        out_specs=pl.BlockSpec(memory_space=pl.ANY),
        scratch_shapes=[
            pltpu.VMEM((S, D), BF16),
            pltpu.VMEM((S, D), BF16),
            pltpu.VMEM((D, 3 * D), BF16),
            pltpu.VMEM((D, D), BF16),
            pltpu.VMEM((2 * D, D), BF16),
            pltpu.VMEM((2, D, D), BF16),
            pltpu.VMEM((DH, DH, H), BF16),
            pltpu.VMEM((D,), BF16),
            pltpu.VMEM((D,), BF16),
            pltpu.VMEM((D,), BF16),
            pltpu.VMEM((D,), BF16),
            pltpu.VMEM((D, D), jnp.int32),
            pltpu.VMEM((D // 2, D), jnp.int32),
            pltpu.VMEM((D // 2, 2 * D), jnp.int32),
            pltpu.VMEM((D // 2, D), jnp.int32),
            pltpu.VMEM((8, 8, D), F32),
            pltpu.VMEM((8, D), F32),
            pltpu.VMEM((2 * D, 128), F32),
            pltpu.VMEM((D, 128), jnp.int32),
            pltpu.VMEM((2 * D, 128), F32),
            pltpu.VMEM((D, D), jnp.int32),
            pltpu.VMEM((2 * D, 128), F32),
            pltpu.VMEM((S, D), F32),
            pltpu.VMEM((S, D), F32),
            pltpu.SemaphoreType.DMA((15,)),
            pltpu.SemaphoreType.DMA((3 * n1,)),
            pltpu.SemaphoreType.DMA(()),
        ],
        compiler_params=pltpu.CompilerParams(vmem_limit_bytes=100 * 1024 * 1024),
        name="hedgehog_s5",
    )(A_x.reshape(S, D), A_wqkv, A_w_phi.transpose(1, 2, 0), A_wo, B_x.reshape(S, D),
      B_Lambda_re, B_Lambda_im, B_B_re, B_B_im, B_C_re, B_C_im, B_log_dt, B_Dskip)
    return out.reshape(1, S, 2 * D)
```

```python
import functools

import jax
import jax.numpy as jnp
from jax import lax
import jax.experimental.pallas as pl
import jax.experimental.pallas.tpu as pltpu

S = 2048
D = 640
H = 32
DH = 20
NG = 8
GR = 80

SB = 512
T = 208
TA = 128
JS = (4, 2)
JB = 2

F32 = jnp.float32
BF16 = jnp.bfloat16
NT = (((1,), (1,)), ((), ()))
NN = (((1,), (0,)), ((), ()))
TN = (((0,), (0,)), ((), ()))


def _dot(a, b, dims=NN):
    return lax.dot_general(a, b, dims, preferred_element_type=F32)


def _ld(ref, r0, r1, cols=slice(None)):
    return pltpu.bitcast(ref[r0 // 2:r1 // 2, cols], BF16)


def _st(ref, r0, val, cols=slice(None)):
    ref[r0 // 2:(r0 + val.shape[0]) // 2, cols] = pltpu.bitcast(val.astype(BF16), jnp.int32)


def _fdiv(x, d):
    return jnp.floor((x.astype(F32) + 0.5) * (1.0 / d)).astype(jnp.int32)


def _tile_rows(i):
    half, j = divmod(i, 5)
    g_lo = (128 * j) // 160
    g_hi = (128 * j + 127) // 160
    return half * 320 + g_lo * GR, (g_hi - g_lo + 1) * GR


def _tile_offsets():
    offs, o = [], 0
    for i in range(10):
        offs.append(o)
        o += _tile_rows(i)[1]
    return offs


TILE_OFF = _tile_offsets()


def _kernel(xa_hbm, wqkv_hbm, wphi_hbm, wo_hbm, xb_hbm, lre_hbm, lim_hbm,
            bre_hbm, bim_hbm, cre_hbm, cim_hbm, ldt_hbm, dsk_hbm,
            out_hbm,
            xa_s, xb_s, wqkv_s, wo_s, b_s, craw_s, wphi_s, p0_s, p1_s, p2_s, p3_s,
            wk_s, wq_s, c_s, phit_s, lam_s, dsk_s, kv_s, kvb_s, z_s,
            b2_s, zb_s, ya_s, yb_s, isem, xsem, osem):
    n1 = S // SB
    T0 = S - 2 * n1 * T

    par_in = (lre_hbm, lim_hbm, ldt_hbm, dsk_hbm)
    par_s = (p0_s, p1_s, p2_s, p3_s)
    par_cp = [pltpu.make_async_copy(r, par_s[k], isem.at[0]) for k, r in enumerate(par_in)]
    wphi_cp = pltpu.make_async_copy(wphi_hbm, wphi_s, isem.at[1])
    xa_cp0 = pltpu.make_async_copy(xb_hbm.at[0:T0], xb_s.at[0:T0], isem.at[2])
    b_cp0, b_cp1 = [], []
    for k, r in enumerate((bre_hbm, bim_hbm)):
        b_cp0.append(pltpu.make_async_copy(
            r.at[0:128 * JB], b_s.at[D * k:D * k + 128 * JB], isem.at[2]))
        b_cp1.append(pltpu.make_async_copy(
            r.at[128 * JB:D], b_s.at[D * k + 128 * JB:D * (k + 1)], isem.at[3]))
    c_cp = [pltpu.make_async_copy(r, craw_s.at[k], isem.at[4])
            for k, r in enumerate((cre_hbm, cim_hbm))]
    wqkv_cp = pltpu.make_async_copy(wqkv_hbm, wqkv_s, isem.at[5])
    wo_cp = pltpu.make_async_copy(wo_hbm, wo_s, isem.at[6])

    def xa_cp(i):
        r = pl.ds(i * SB if isinstance(i, int) else pl.multiple_of(i * SB, SB), SB)
        return pltpu.make_async_copy(xa_hbm.at[r], xa_s.at[r], xsem.at[i])

    def ssm_rows(blk):
        r0 = T0 + blk * T
        return pl.ds(r0 if isinstance(r0, int) else pl.multiple_of(r0, 16), T)

    def xb_cp(blk):
        r = ssm_rows(blk)
        return pltpu.make_async_copy(xb_hbm.at[r], xb_s.at[r], xsem.at[blk])

    r2 = pl.ds(T0 + n1 * T, n1 * T)
    xb2_cp = pltpu.make_async_copy(xb_hbm.at[r2], xb_s.at[r2], isem.at[6])

    for cp in par_cp + [wphi_cp, xa_cp0] + b_cp0:
        cp.start()

    for cp in par_cp:
        cp.wait()
    for cp in b_cp1:
        cp.start()
    lre = par_s[0][...].astype(F32).reshape(1, D)
    lim = par_s[1][...].astype(F32).reshape(1, D)
    dt = jnp.exp(par_s[2][...].astype(F32).reshape(1, D)).astype(BF16).astype(F32)
    dsk_s[...] = jnp.broadcast_to(par_s[3][...].astype(F32).reshape(1, D), (8, D))
    ar = dt * lre
    ai = dt * lim
    kk = (lax.broadcasted_iota(jnp.int32, (8, D), 0) + 1).astype(F32)
    mag = jnp.exp(kk * ar)
    t_re = mag * jnp.cos(kk * ai)
    t_im = mag * jnp.sin(kk * ai)
    row = lax.broadcasted_iota(jnp.int32, (8, D), 0)
    for n, (sh, keep) in enumerate(((1, row == 0), (1, row >= 1), (2, row >= 2), (4, row >= 4))):
        lam_s[2 * n] = jnp.where(keep, jnp.broadcast_to(t_re[sh - 1:sh], (8, D)), 0.0)
        lam_s[2 * n + 1] = jnp.where(keep, jnp.broadcast_to(t_im[sh - 1:sh], (8, D)), 0.0)
    l_re = t_re[0:1]
    l_im = t_im[0:1]
    inv = 1.0 / (lre * lre + lim * lim)
    nr = l_re - 1.0
    co_re = 2.0 * (nr * lre + l_im * lim) * inv
    co_im = 2.0 * (l_im * lre - nr * lim) * inv

    wphi_cp.wait()
    for cp in c_cp:
        cp.start()

    def prep_phi():
        lcat = jnp.concatenate([wphi_s[d].astype(F32) for d in range(DH)], axis=1)
        lcat = lcat.astype(BF16)
        r_i = lax.broadcasted_iota(jnp.int32, (GR, 128), 0)
        l_i = lax.broadcasted_iota(jnp.int32, (GR, 128), 1)
        e_g = jnp.where((r_i >> 2)[:, 0:DH] == l_i[:, 0:DH], 1.0, 0.0).astype(BF16)
        hl_r = r_i & 3
        k_i = lax.broadcasted_iota(jnp.int32, (D, 128), 0)
        for ct in range(5):
            cc = lax.broadcasted_iota(jnp.int32, (8, 128), 1) + 128 * ct
            h_c = _fdiv(cc, DH)
            tgt = 32 * (cc - DH * h_c) + h_c
            pm = jnp.where(k_i == tgt[0:1], 1.0, 0.0).astype(BF16)
            x_t = _dot(lcat, pm).astype(BF16)
            rep = _dot(e_g, x_t)
            for g in range((128 * ct) // GR, (128 * ct + 127) // GR + 1):
                _st(phit_s, g * GR, jnp.where(hl_r + 4 * g == h_c[0:1], rep, 0.0),
                    slice(128 * ct, 128 * (ct + 1)))

    prep_phi()

    def fold(col0, dst):
        acc = [None] * NG
        for kt in range(5):
            g_lo = (128 * kt) // GR
            g_hi = (128 * kt + 127) // GR
            part = _dot(_ld(phit_s, g_lo * GR, (g_hi + 1) * GR, slice(128 * kt, 128 * (kt + 1))),
                        wqkv_s[:, col0 + 128 * kt:col0 + 128 * (kt + 1)], NT)
            for g in range(g_lo, g_hi + 1):
                p = part[(g - g_lo) * GR:(g - g_lo + 1) * GR]
                acc[g] = p if acc[g] is None else acc[g] + p
        for g, a in enumerate(acc):
            _st(dst, g * GR, a)

    def prep_c():
        for j in range(5):
            cs = slice(128 * j, 128 * (j + 1))
            cr_ = co_re[:, cs]
            ci_ = co_im[:, cs]
            ncr_ = -cr_
            for r in range(5):
                rs = slice(128 * r, 128 * (r + 1))
                a = craw_s[0, rs, cs].astype(F32)
                b = craw_s[1, rs, cs].astype(F32)
                _st(c_s, 128 * r, cr_ * a - ci_ * b, slice(256 * j, 256 * j + 128))
                _st(c_s, 128 * r, ncr_ * b - ci_ * a, slice(256 * j + 128, 256 * j + 256))

    def features(p):
        ps = [p[8 * k:8 * k + 8] for k in range(10)]
        mx = functools.reduce(jnp.maximum, ps)
        mn = functools.reduce(jnp.minimum, ps)
        mx = jnp.maximum(mx, pltpu.roll(mx, 4, 0))
        mn = jnp.minimum(mn, pltpu.roll(mn, 4, 0))
        ep = [jnp.exp(q - mx) for q in ps]
        en = [jnp.exp(mn - q) for q in ps]
        sp = functools.reduce(jnp.add, ep)
        sn = functools.reduce(jnp.add, en)
        sp = sp + pltpu.roll(sp, 4, 0)
        sn = sn + pltpu.roll(sn, 4, 0)
        return ep, en, sp, sn

    def k_proj(i):
        x = xa_s[pl.ds(pl.multiple_of(i * SB, SB), SB), :]
        return _dot(_ld(wk_s, 0, 2 * D), x, NT)

    def k_side(pkv):
        vt = pkv[D:].astype(BF16)
        rows = []
        for g in range(NG):
            ep, en, sp, sn = features(pkv[g * GR:(g + 1) * GR])
            rp = 1.0 / sp
            rn = 1.0 / sn
            rows += [e * rp for e in ep] + [e * rn for e in en]
        phi = jnp.concatenate(rows, axis=0)
        zs = phi[:, 0:128]
        for c in range(1, SB // 128):
            zs = zs + phi[:, 128 * c:128 * (c + 1)]
        z_s[...] += zs
        phib = phi.astype(BF16)
        for t in range(10):
            r0, nr_ = _tile_rows(t)
            kv_s[TILE_OFF[t]:TILE_OFF[t] + nr_, :] += _dot(
                vt[r0:r0 + nr_], phib[128 * t:128 * (t + 1)], NT)

    def finalize_kv():
        z = jnp.sum(z_s[...], axis=1, keepdims=True)
        zb_s[...] = jnp.broadcast_to(z, z_s.shape)
        for t in range(10):
            r0, nr_ = _tile_rows(t)
            rr = lax.broadcasted_iota(jnp.int32, (nr_, 128), 0) + r0
            cc = lax.broadcasted_iota(jnp.int32, (nr_, 128), 1) + 128 * t
            h_row = _fdiv(rr, DH)
            h_col = 4 * _fdiv(cc, 160) + (cc & 3)
            _st(kvb_s, TILE_OFF[t], jnp.where(
                h_row == h_col, kv_s[TILE_OFF[t]:TILE_OFF[t] + nr_, :], 0.0))

    def q_proj(i):
        x = xa_s[pl.ds(pl.multiple_of(i * SB, SB), SB), :]
        return _dot(_ld(wq_s, 0, D), x, NT)

    def q_side(i, pq):
        r0_ = pl.multiple_of(i * SB, SB)
        rows = []
        nl = SB // 128
        for g in range(NG):
            ep, en, sp, sn = features(pq[g * GR:(g + 1) * GR])
            zb = zb_s[g * 160:(g + 1) * 160, :]
            zb = jnp.concatenate([zb] * nl, axis=1) if nl > 1 else zb
            dp = functools.reduce(jnp.add, [ep[k] * zb[8 * k:8 * k + 8] for k in range(10)])
            dn = functools.reduce(jnp.add, [en[k] * zb[80 + 8 * k:88 + 8 * k] for k in range(10)])
            dd = dp / sp + dn / sn
            den = dd + pltpu.roll(dd, 4, 0) + 1e-6
            rp = 1.0 / (sp * den)
            rn = 1.0 / (sn * den)
            rows += [e * rp for e in ep] + [e * rn for e in en]
        phib = jnp.concatenate(rows, axis=0).astype(BF16)
        acc = [None] * NG
        for t in range(10):
            r0, nr_ = _tile_rows(t)
            part = _dot(_ld(kvb_s, TILE_OFF[t], TILE_OFF[t] + nr_), phib[128 * t:128 * (t + 1)])
            for k in range(nr_ // GR):
                g = r0 // GR + k
                p = part[k * GR:(k + 1) * GR]
                acc[g] = p if acc[g] is None else acc[g] + p
        ot = jnp.concatenate(acc, axis=0).astype(BF16)
        for c in range(nl):
            rc = pl.ds(pl.multiple_of(r0_ + 128 * c, 128), 128)
            ya_s[rc, :] = _dot(ot[:, 128 * c:128 * (c + 1)], wo_s[...], TN)
            pltpu.make_async_copy(ya_s.at[rc], out_hbm.at[rc, pl.ds(0, D)], osem).start()

    def ssm_w(xb, j):
        return _dot(xb, _ld(b2_s, 256 * j, 256 * (j + 1)), NT)

    def pack_b(j):
        _st(b2_s, 256 * j, b_s[128 * j:128 * (j + 1), :])
        _st(b2_s, 256 * j + 128, b_s[D + 128 * j:D + 128 * (j + 1), :])

    def ssm_scan(w, j, carry):
        tb = w.shape[0]
        cs = slice(128 * j, 128 * (j + 1))
        tab = [lam_s[n, :, cs] for n in range(8)]
        c_re, c_im = carry[2 * j], carry[2 * j + 1]
        o_re, o_im = [], []
        for r in range(tb // 8):
            u_re = w[8 * r:8 * r + 8, 0:128]
            u_im = w[8 * r:8 * r + 8, 128:256]
            for n, sh in enumerate((1, 1, 2, 4)):
                m_re, m_im = tab[2 * n], tab[2 * n + 1]
                s_re = pltpu.roll(c_re if n == 0 else u_re, sh, 0)
                s_im = pltpu.roll(c_im if n == 0 else u_im, sh, 0)
                u_re = u_re + (m_re * s_re - m_im * s_im)
                u_im = u_im + (m_re * s_im + m_im * s_re)
            c_re, c_im = u_re, u_im
            o_re.append(u_re)
            o_im.append(u_im)
        carry = carry[:2 * j] + (c_re, c_im) + carry[2 * j + 2:]
        return [jnp.concatenate(o_re, 0).astype(BF16),
                jnp.concatenate(o_im, 0).astype(BF16)], carry

    def ssm_scan_all(ws, carry):
        s_tiles = []
        for j in range(5):
            st, carry = ssm_scan(ws[j], j, carry)
            s_tiles += st
        return jnp.concatenate(s_tiles, axis=1), carry

    def ssm_back(s, rows, ksplit=False):
        y = xb_s[rows, :].astype(F32) * dsk_s[0:1, :]
        if ksplit:
            for j in range(5):
                y = y + _dot(s[:, 256 * j:256 * (j + 1)], _ld(c_s, 0, D, slice(256 * j, 256 * (j + 1))), NT)
        else:
            y = y + _dot(s, _ld(c_s, 0, D), NT)
        yb_s[rows, :] = y

    def ssm_out(rows):
        pltpu.make_async_copy(yb_s.at[rows], out_hbm.at[rows, pl.ds(D, D)], osem).start()

    zero = jnp.zeros((8, 128), F32)
    carry = (zero,) * 10
    rows0 = pl.ds(0, T0)
    xa_cp0.wait()
    for cp in b_cp0:
        cp.wait()
    wqkv_cp.start()
    xb0 = xb_s[rows0, :]
    for j in range(JB):
        pack_b(j)
    w0 = [ssm_w(xb0, j) for j in range(JB)]
    for cp in b_cp1:
        cp.wait()
    xa_cp(0).start()
    xb_cp(0).start()
    for j in range(JB, 5):
        pack_b(j)
    w0 += [ssm_w(xb0, j) for j in range(JB, 5)]
    parts = [(0, TA), (TA, T0)]
    st = {}

    def scan_part(j, p, carry):
        lo, hi = parts[p]
        st[j, p], carry = ssm_scan(w0[j][lo:hi], j, carry)
        return carry

    early = [(j, p) for j in range(5) for p in range(2) if j < JS[p]]
    for j, p in early:
        carry = scan_part(j, p, carry)
    for cp in c_cp:
        cp.wait()
    prep_c()
    for j in range(5):
        for p in range(2):
            if (j, p) not in early:
                carry = scan_part(j, p, carry)
    for p, (lo, hi) in enumerate(parts):
        ssm_back(jnp.concatenate([t for j in range(5) for t in st[j, p]], axis=1),
                 pl.ds(lo, hi - lo), ksplit=True)
    kv_s[...] = jnp.zeros(kv_s.shape, F32)
    z_s[...] = jnp.zeros(z_s.shape, F32)
    ssm_out(pl.ds(0, T0))
    wqkv_cp.wait()
    wo_cp.start()
    for i in range(1, n1):
        xa_cp(i).start()
        xb_cp(i).start()
    fold(0, wq_s)
    fold(D, wk_s)
    _st(wk_s, D, wqkv_s[:, 2 * D:3 * D].T)
    xb2_cp.start()

    def body1(i, carry):
        xa_cp(i).wait()
        xb_cp(i).wait()
        rows = ssm_rows(i)
        ws = [ssm_w(xb_s[rows, :], j) for j in range(5)]
        pkv = k_proj(i)
        s, carry = ssm_scan_all(ws, carry)
        ssm_back(s, rows)
        k_side(pkv)
        ssm_out(rows)
        return carry

    carry = lax.fori_loop(0, n1, body1, carry)
    wo_cp.wait()
    xb2_cp.wait()

    def body2(i, carry):
        rows = ssm_rows(i + n1)
        ws = [ssm_w(xb_s[rows, :], j) for j in range(5)]
        pq = q_proj(i)
        finalize_kv()
        s, carry = ssm_scan_all(ws, carry)
        ssm_back(s, rows)
        ssm_out(rows)
        q_side(i, pq)
        return carry

    lax.fori_loop(0, n1, body2, carry)
    pltpu.make_async_copy(out_hbm, out_hbm, osem).wait()


@jax.jit
def pallas_concat_heads__linear_kernel_hedgehog__ssm_conv_s5__prompt_kernel(
      A_x, A_wqkv, A_w_phi, A_wo, B_x, B_Lambda_re, B_Lambda_im, B_B_re, B_B_im,
      B_C_re, B_C_im, B_log_dt, B_Dskip):
    n1 = S // SB
    out = pl.pallas_call(
        _kernel,
        out_shape=jax.ShapeDtypeStruct((S, 2 * D), F32),
        in_specs=[pl.BlockSpec(memory_space=pl.ANY)] * 13,
        out_specs=pl.BlockSpec(memory_space=pl.ANY),
        scratch_shapes=[
            pltpu.VMEM((S, D), BF16),
            pltpu.VMEM((S, D), BF16),
            pltpu.VMEM((D, 3 * D), BF16),
            pltpu.VMEM((D, D), BF16),
            pltpu.VMEM((2 * D, D), BF16),
            pltpu.VMEM((2, D, D), BF16),
            pltpu.VMEM((DH, DH, H), BF16),
            pltpu.VMEM((D,), BF16),
            pltpu.VMEM((D,), BF16),
            pltpu.VMEM((D,), BF16),
            pltpu.VMEM((D,), BF16),
            pltpu.VMEM((D, D), jnp.int32),
            pltpu.VMEM((D // 2, D), jnp.int32),
            pltpu.VMEM((D // 2, 2 * D), jnp.int32),
            pltpu.VMEM((D // 2, D), jnp.int32),
            pltpu.VMEM((8, 8, D), F32),
            pltpu.VMEM((8, D), F32),
            pltpu.VMEM((2 * D, 128), F32),
            pltpu.VMEM((D, 128), jnp.int32),
            pltpu.VMEM((2 * D, 128), F32),
            pltpu.VMEM((D, D), jnp.int32),
            pltpu.VMEM((2 * D, 128), F32),
            pltpu.VMEM((S, D), F32),
            pltpu.VMEM((S, D), F32),
            pltpu.SemaphoreType.DMA((7,)),
            pltpu.SemaphoreType.DMA((n1,)),
            pltpu.SemaphoreType.DMA(()),
        ],
        compiler_params=pltpu.CompilerParams(vmem_limit_bytes=100 * 1024 * 1024),
        name="hedgehog_s5",
    )(A_x.reshape(S, D), A_wqkv, A_w_phi.transpose(1, 2, 0), A_wo, B_x.reshape(S, D),
      B_Lambda_re, B_Lambda_im, B_B_re, B_B_im, B_C_re, B_C_im, B_log_dt, B_Dskip)
    return out.reshape(1, S, 2 * D)
```
